```python
import jax
import jax.numpy as jnp

def _softmax(x, axis=-1):
    return jax.nn.softmax(x, axis=axis)
def _gelu(x):
    return jax.nn.gelu(x, approximate=True)
def _silu(x):
    return jax.nn.silu(x)
def _sigmoid(x):
    return jax.nn.sigmoid(x)
def _layernorm(x, axis=-1, eps=1e-5):
    m = jnp.mean(x, axis=axis, keepdims=True)
    v = jnp.var(x, axis=axis, keepdims=True)
    return (x - m) / jnp.sqrt(v + eps)
def _scatter_add(tgt, idx, src, axis=0):
    return tgt.at[idx].add(src)
def _segment_sum(src, seg, n):
    return jax.ops.segment_sum(src, seg, n)
class _Rng:
    def __init__(self, key):
        self._k = key
    def _next(self):
        self._k, sub = jax.random.split(self._k)
        return sub
    def normal(self, shape):
        return jax.random.normal(self._next(), shape, dtype=jnp.bfloat16)
    def randint(self, lo, hi, shape):
        return jax.random.randint(self._next(), shape, lo, hi, dtype=jnp.int32)
    def uniform(self, shape, lo=0.0, hi=1.0):
        return jax.random.uniform(self._next(), shape, jnp.bfloat16, lo, hi)
    def permutation(self, n):
        return jax.random.permutation(self._next(), n)


kernel_name = 'gated_mix__sliding_block_cached__mixer_s_mlp__decode'

def setup_inputs():
    _rng = _Rng(jax.random.key(int.from_bytes(__import__("os").urandom(4), "little")))
    _w = (lambda a: (lambda t: t.astype(jnp.bfloat16) if jnp.issubdtype(t.dtype, jnp.floating) else t)(jnp.asarray(a)))
    def _A_setup():
        B, Sq, D = 1, 1, 576
        Hq, Hkv, Sk, Dh = 32, 16, 65536, 128
        assert Hq % Hkv == 0, (Hq, Hkv)
        return {
            "x": _w((lambda *s: _rng.normal(s) * 0.05)(B, Sq, D)),
            "k_cache": _w((lambda *s: _rng.normal(s) * 0.05)(B, Hkv, Sk, Dh)),
            "v_cache": _w((lambda *s: _rng.normal(s) * 0.05)(B, Hkv, Sk, Dh)),
            "wq": _w((lambda *s: _rng.normal(s) * 0.05)(D, Hq * Dh) * (D ** -0.5)),
            "wo": _w((lambda *s: _rng.normal(s) * 0.05)(Hq * Dh, D) * ((Hq * Dh) ** -0.5)),
        }
    _A_in = _A_setup()

    def _B_setup():
        B, S, D, F = 1, 1, 576, 4608
        return {
            "x":  _w((lambda *s: _rng.normal(s) * 0.05)(B, S, D)),
            "w1": _w((lambda *s: _rng.normal(s) * 0.05)(D, D) * (D ** -0.5)),
            "w2": _w((lambda *s: _rng.normal(s) * 0.05)(D, D) * (D ** -0.5)),
            "w3": _w((lambda *s: _rng.normal(s) * 0.05)(D, F) * (D ** -0.5)),
            "w4": _w((lambda *s: _rng.normal(s) * 0.05)(F, D) * (F ** -0.5)),
        }
    _B_in = _B_setup()

    return {
        "A_x": _A_in["x"],
        "A_k_cache": _A_in["k_cache"],
        "A_v_cache": _A_in["v_cache"],
        "A_wq": _A_in["wq"],
        "A_wo": _A_in["wo"],
        "B_x": _B_in["x"],
        "B_w1": _B_in["w1"],
        "B_w2": _B_in["w2"],
        "B_w3": _B_in["w3"],
        "B_w4": _B_in["w4"],
        "gate_w": _w((lambda *s: _rng.normal(s) * 0.05)(576)),
    }

def reference(A_x, A_k_cache, A_v_cache, A_wq, A_wo, B_x, B_w1, B_w2, B_w3, B_w4, gate_w):
    def _A_ref(x, k_cache, v_cache, wq, wo):
        B, Sq, D = x.shape
        Hq, Dh = 32, 128
        Hkv, Sk = k_cache.shape[1], k_cache.shape[2]
        W = min(4096, max(256, Sk // 4))
        rep = Hq // Hkv
        q = (lambda x, *d: x.transpose(*d))((x @ wq).reshape(B, Sq, Hq, Dh), 0, 2, 1, 3)
        k = jnp.repeat(k_cache[:, :, Sk - W:, :], rep, axis=1)
        v = jnp.repeat(v_cache[:, :, Sk - W:, :], rep, axis=1)
        scores = jnp.einsum("bhqd,bhkd->bhqk", q, k) * (Dh ** -0.5)
        p = _softmax(scores, axis=-1)
        o = jnp.einsum("bhqk,bhkd->bhqd", p, v)
        return (lambda x, *d: x.transpose(*d))(o, 0, 2, 1, 3).reshape(B, Sq, Hq * Dh) @ wo

    def _B_ref(x, w1, w2, w3, w4):
        B, S, D = x.shape
        h = _gelu(_layernorm(x, axis=-1) @ w1)
        c = D // 4
        g0 = jnp.pad(h[:, :, 0*c:1*c], ((0, 0), (1, 0), (0, 0)))[:, :S, :]
        g1 = jnp.pad(h[:, :, 1*c:2*c], ((0, 0), (0, 1), (0, 0)))[:, 1:, :]
        g2 = jnp.pad(h[:, :, 2*c:3*c], ((0, 0), (2, 0), (0, 0)))[:, :S, :]
        g3 = jnp.pad(h[:, :, 3*c:   ], ((0, 0), (0, 2), (0, 0)))[:, 2:, :]
        hs = jnp.concatenate([g0, g1, g2, g3], axis=-1) @ w2
        x1 = x + hs
        h2 = _gelu(_layernorm(x1, axis=-1) @ w3) @ w4
        return x1 + h2

    x = A_x
    g = _sigmoid((x * gate_w).sum(-1, keepdims=True))
    a = _A_ref(x, A_k_cache, A_v_cache, A_wq, A_wo)
    b = _B_ref(x, B_w1, B_w2, B_w3, B_w4)
    return g * a + (1 - g) * b
```

```python
import functools

import jax
import jax.numpy as jnp
from jax import lax
import jax.experimental.pallas as pl
import jax.experimental.pallas.tpu as pltpu

_ROWS = 8
_HEAD_GROUP = 4
_MLP_CHUNK = 512
_WO_SPLITS = (12, 3, 1)

_NT = (((1,), (1,)), ((), ()))


def _dot(a, b):
    return jnp.dot(a, b, preferred_element_type=jnp.float32)


def _dot_nt(a, b):
    return lax.dot_general(a, b, _NT, preferred_element_type=jnp.float32)


def _kernel(
    ax_hbm, bx_hbm, gw_hbm, k_hbm, v_hbm, wq_hbm, wot_hbm, w3_hbm, w4t_hbm,
    out_ref,
    ax_buf, bx_buf, gw_buf, k_buf, v_buf, wq_buf, wot_buf, w3_buf, w4t_buf,
    q_buf, o_buf, h_buf, sems,
    *, window,
):
    f32, bf16 = jnp.float32, jnp.bfloat16
    hkv, _, dh = k_buf.shape
    d = wq_buf.shape[0]
    ff = w3_buf.shape[1]
    pair = 2 * dh
    start = k_hbm.shape[2] - window
    n_groups = hkv // _HEAD_GROUP

    def copy(src, dst, sem):
        return pltpu.make_async_copy(src, dst, sems.at[sem])

    def kv_copies(g):
        heads = pl.ds(g * _HEAD_GROUP, _HEAD_GROUP)
        rows = pl.ds(start, window)
        return (
            copy(k_hbm.at[0, heads, rows, :], k_buf.at[heads], 3 + g),
            copy(v_hbm.at[0, heads, rows, :], v_buf.at[heads], 3 + g),
        )

    first = (
        copy(wq_hbm, wq_buf, 0),
        copy(ax_hbm, ax_buf, 0),
        copy(bx_hbm, bx_buf, 0),
        copy(gw_hbm, gw_buf, 0),
    )
    w3_copy = copy(w3_hbm, w3_buf, 1)
    w4_copy = copy(w4t_hbm, w4t_buf, 2)
    wo_copies = []
    h0 = 0
    for i, n in enumerate(_WO_SPLITS):
        cols = pl.ds(h0 * pair, n * pair)
        wo_copies.append(
            (h0, n, copy(wot_hbm.at[:, cols], wot_buf.at[:, cols], 3 + n_groups + i))
        )
        h0 += n

    for c in first:
        c.start()
    w3_copy.start()
    w4_copy.start()
    for g in range(n_groups):
        for c in kv_copies(g):
            c.start()
    for _, _, c in wo_copies:
        c.start()

    for c in first:
        c.wait()
    ax = ax_buf[0]
    bx = bx_buf[0].astype(f32)
    logit = jnp.sum(
        ax.astype(f32) * gw_buf[...].astype(f32).reshape(1, d), axis=-1, keepdims=True
    )
    gate = jax.nn.sigmoid(logit)
    ax_rows = jnp.broadcast_to(ax.astype(f32), (_ROWS, d)).astype(bf16)

    def q_step(i, carry):
        cols = pl.ds(pl.multiple_of(i * _MLP_CHUNK, _MLP_CHUNK), _MLP_CHUNK)
        q_buf[:, cols] = _dot(ax_rows, wq_buf[:, cols])
        return carry

    lax.fori_loop(0, hkv * pair // _MLP_CHUNK, q_step, None)

    centered = bx - jnp.mean(bx, axis=-1, keepdims=True)
    var = jnp.mean(centered * centered, axis=-1, keepdims=True)
    normed = centered / jnp.sqrt(var + 1e-5)
    normed_rows = jnp.broadcast_to(normed, (_ROWS, d)).astype(bf16)

    w3_copy.wait()

    def up_step(i, carry):
        cols = pl.ds(pl.multiple_of(i * _MLP_CHUNK, _MLP_CHUNK), _MLP_CHUNK)
        h_buf[:, cols] = jax.nn.gelu(
            _dot(normed_rows, w3_buf[:, cols]), approximate=True
        )
        return carry

    lax.fori_loop(0, ff // _MLP_CHUNK, up_step, None)
    w4_copy.wait()

    def down_step(i, acc):
        cols = pl.ds(pl.multiple_of(i * _MLP_CHUNK, _MLP_CHUNK), _MLP_CHUNK)
        return acc + _dot_nt(h_buf[:, cols].astype(bf16), w4t_buf[:, cols])

    mlp = lax.fori_loop(0, ff // _MLP_CHUNK, down_step, jnp.zeros((_ROWS, d), f32))
    b_gated = (1.0 - gate) * (bx + mlp[0:1])

    row = lax.broadcasted_iota(jnp.int32, (_ROWS, dh), 0)
    scale = dh ** -0.5

    def head_step(h, carry):
        @pl.when(h % _HEAD_GROUP == 0)
        def _():
            for c in kv_copies(h // _HEAD_GROUP):
                c.wait()

        c0 = pl.multiple_of(h * pair, pair)
        c1 = pl.multiple_of(h * pair + dh, dh)
        q = jnp.where(row == 0, q_buf[:, pl.ds(c0, dh)], q_buf[:, pl.ds(c1, dh)])
        s = _dot_nt(q.astype(bf16), k_buf[h]) * scale
        e = jnp.exp(s - jnp.max(s, axis=-1, keepdims=True))
        denom = jnp.sum(e, axis=-1, keepdims=True)
        o = _dot(e.astype(bf16), v_buf[h]) / denom
        o_buf[:, pl.ds(c0, dh)] = jnp.where(row == 0, o, 0.0)
        o_buf[:, pl.ds(c1, dh)] = jnp.where(row == 1, o, 0.0)
        return carry

    lax.fori_loop(0, hkv, head_step, None)

    def wo_step(h, acc):
        cols = pl.ds(pl.multiple_of(h * pair, pair), pair)
        return acc + _dot_nt(o_buf[:, cols].astype(bf16), wot_buf[:, cols])

    acc = jnp.zeros((_ROWS, d), f32)
    for h0, n, c in wo_copies:
        c.wait()
        if n == 1:
            acc = wo_step(h0, acc)
        else:
            acc = lax.fori_loop(h0, h0 + n, wo_step, acc)

    attn = acc[0:1] + acc[1:2]
    out_ref[0] = (gate * attn + b_gated).astype(out_ref.dtype)


@jax.jit
def pallas_gated_mix__sliding_block_cached__mixer_s_mlp__decode_kernel(
    A_x: jax.Array,
    A_k_cache: jax.Array,
    A_v_cache: jax.Array,
    A_wq: jax.Array,
    A_wo: jax.Array,
    B_x: jax.Array,
    B_w1: jax.Array,
    B_w2: jax.Array,
    B_w3: jax.Array,
    B_w4: jax.Array,
    gate_w: jax.Array,
):
    del B_w1, B_w2
    b, sq, d = A_x.shape
    _, hkv, sk, dh = A_k_cache.shape
    ff = B_w3.shape[1]
    assert (b, sq) == (1, 1) and B_x.shape == A_x.shape
    assert A_wq.shape == (d, 2 * hkv * dh) and sum(_WO_SPLITS) == hkv
    window = min(4096, max(256, sk // 4))
    n_sems = 3 + hkv // _HEAD_GROUP + len(_WO_SPLITS)
    dt = A_x.dtype

    wot, w4t = A_wo.T, B_w4.T
    hbm = pl.BlockSpec(memory_space=pltpu.HBM)
    return pl.pallas_call(
        functools.partial(_kernel, window=window),
        out_shape=jax.ShapeDtypeStruct(A_x.shape, dt),
        in_specs=[hbm] * 9,
        out_specs=pl.BlockSpec(memory_space=pltpu.VMEM),
        scratch_shapes=[
            pltpu.VMEM(A_x.shape, dt),
            pltpu.VMEM(B_x.shape, dt),
            pltpu.VMEM(gate_w.shape, dt),
            pltpu.VMEM((hkv, window, dh), dt),
            pltpu.VMEM((hkv, window, dh), dt),
            pltpu.VMEM(A_wq.shape, dt),
            pltpu.VMEM(wot.shape, dt),
            pltpu.VMEM(B_w3.shape, dt),
            pltpu.VMEM(w4t.shape, dt),
            pltpu.VMEM((_ROWS, A_wq.shape[1]), jnp.float32),
            pltpu.VMEM((_ROWS, A_wq.shape[1]), jnp.float32),
            pltpu.VMEM((_ROWS, ff), jnp.float32),
            pltpu.SemaphoreType.DMA((n_sems,)),
        ],
        compiler_params=pltpu.CompilerParams(vmem_limit_bytes=100 * 2**20),
    )(A_x, B_x, gate_w, A_k_cache, A_v_cache, A_wq, wot, B_w3, w4t)
```

```python
import jax
import jax.numpy as jnp
from jax import lax
import jax.experimental.pallas as pl
import jax.experimental.pallas.tpu as pltpu

_ROWS = 8
_CHUNK = 512

_W4_PIECES = (
    (0, 576, 0, 2560),
    (0, 576, 2560, 1024),
    (256, 320, 3584, 1024),
    (128, 128, 3584, 1024),
    (0, 128, 3584, 512),
    (0, 128, 4096, 512),
)


def _dot(a, b):
    return jnp.dot(a, b, preferred_element_type=jnp.float32)


def _dot_nt(a, b):
    return lax.dot_general(
        a, b, (((1,), (1,)), ((), ())), preferred_element_type=jnp.float32
    )


def _kernel(
    x_hbm, gw_hbm, k_hbm, v_hbm, wq_hbm, wot_hbm, w3_hbm, w4t_hbm,
    out_ref,
    x_buf, gw_buf, k_buf, v_buf, wq_buf, wot_buf, w3_buf,
    q_buf, o_buf, h_buf, acc_buf, last_sem, *w4_bufs,
):
    f32, bf16 = jnp.float32, jnp.bfloat16
    hkv, window, dh = k_buf.shape
    d, ff = w3_buf.shape
    pair = 2 * dh

    def w4_copy(i, sem):
        r0, nr, c0, nc = _W4_PIECES[i]
        src = w4t_hbm.at[pl.ds(r0, nr), pl.ds(c0, nc)]
        return pltpu.make_async_copy(src, w4_bufs[i], sem)

    def mlp_down(i, copy):
        r0, nr, c0, nc = _W4_PIECES[i]
        hidden = h_buf[:, c0:c0 + nc].astype(bf16)
        partial = acc_buf[:, r0:r0 + nr]
        copy.wait()
        total = partial + _dot_nt(hidden, w4_bufs[i][...])
        if c0 + nc == ff:
            out_ref[0, :, r0:r0 + nr] = total[0:1].astype(out_ref.dtype)
        else:
            acc_buf[:, r0:r0 + nr] = total

    def chunk(i):
        return pl.ds(pl.multiple_of(i * _CHUNK, _CHUNK), _CHUNK)

    n_early = len(_W4_PIECES) - 1
    last_copy = w4_copy(n_early, last_sem)

    def all_but_last_piece(sems):
        def copy(src, dst, i):
            return pltpu.make_async_copy(src, dst, sems.at[i])

        recent = pl.ds(k_hbm.shape[2] - window, window)
        q_copies = (
            copy(wq_hbm, wq_buf, 0),
            copy(x_hbm, x_buf, 0),
            copy(gw_hbm, gw_buf, 0),
        )
        kv_copies = (
            copy(k_hbm.at[0, :, recent, :], k_buf, 1),
            copy(v_hbm.at[0, :, recent, :], v_buf, 1),
        )
        proj_copies = (copy(wot_hbm, wot_buf, 2), copy(w3_hbm, w3_buf, 2))
        w4_copies = [w4_copy(i, sems.at[3 + i]) for i in range(n_early)]
        for c in (*q_copies, *kv_copies, *proj_copies, *w4_copies, last_copy):
            c.start()

        for c in q_copies:
            c.wait()
        x = x_buf[0].astype(f32)
        gw = gw_buf[...].astype(f32).reshape(1, d)
        gate = jax.nn.sigmoid(jnp.sum(x * gw, axis=-1, keepdims=True))

        centered = x - jnp.mean(x, axis=-1, keepdims=True)
        var = jnp.mean(centered * centered, axis=-1, keepdims=True)
        normed = centered / jnp.sqrt(var + 1e-5)
        normed_rows = jnp.broadcast_to(normed, (_ROWS, d)).astype(bf16)
        x_rows = jnp.broadcast_to(x, (_ROWS, d)).astype(bf16)

        def q_step(i, carry):
            q_buf[:, chunk(i)] = _dot(x_rows, wq_buf[:, chunk(i)])
            return carry

        lax.fori_loop(0, hkv * pair // _CHUNK, q_step, None)

        for c in kv_copies:
            c.wait()
        row = lax.broadcasted_iota(jnp.int32, (_ROWS, dh), 0)

        def head_step(h, carry):
            even = pl.ds(pl.multiple_of(h * pair, pair), dh)
            odd = pl.ds(pl.multiple_of(h * pair + dh, dh), dh)
            q = jnp.where(row == 0, q_buf[:, even], q_buf[:, odd])
            s = _dot_nt(q.astype(bf16), k_buf[h]) * dh ** -0.5
            e = jnp.exp(s - jnp.max(s, axis=-1, keepdims=True))
            denom = jnp.sum(e, axis=-1, keepdims=True)
            o = _dot(e.astype(bf16), v_buf[h]) / denom
            o_buf[:, even] = jnp.where(row == 0, o, 0.0)
            o_buf[:, odd] = jnp.where(row == 1, o, 0.0)
            return carry

        lax.fori_loop(0, hkv, head_step, None)

        for c in proj_copies:
            c.wait()

        def wo_step(i, acc):
            return acc + _dot_nt(o_buf[:, chunk(i)].astype(bf16), wot_buf[:, chunk(i)])

        attn = lax.fori_loop(
            0, hkv * pair // _CHUNK, wo_step, jnp.zeros((_ROWS, d), f32)
        )
        mixed = gate * (attn[0:1] + attn[1:2]) + (1.0 - gate) * x
        acc_buf[...] = jnp.broadcast_to(mixed, (_ROWS, d))

        def up_step(i, carry):
            pre = _dot(normed_rows, w3_buf[:, chunk(i)])
            h_buf[:, chunk(i)] = (1.0 - gate) * jax.nn.gelu(pre, approximate=True)
            return carry

        lax.fori_loop(0, ff // _CHUNK, up_step, None)
        for i, c in enumerate(w4_copies):
            mlp_down(i, c)

    pl.run_scoped(all_but_last_piece, pltpu.SemaphoreType.DMA((3 + n_early,)))
    mlp_down(n_early, last_copy)


@jax.jit
def pallas_gated_mix__sliding_block_cached__mixer_s_mlp__decode_kernel(
    A_x: jax.Array,
    A_k_cache: jax.Array,
    A_v_cache: jax.Array,
    A_wq: jax.Array,
    A_wo: jax.Array,
    B_x: jax.Array,
    B_w1: jax.Array,
    B_w2: jax.Array,
    B_w3: jax.Array,
    B_w4: jax.Array,
    gate_w: jax.Array,
):
    del B_x, B_w1, B_w2
    b, sq, d = A_x.shape
    _, hkv, sk, dh = A_k_cache.shape
    ff = B_w3.shape[1]
    hidden = 2 * hkv * dh
    assert (b, sq) == (1, 1)
    assert A_wq.shape == (d, hidden) and hidden % _CHUNK == 0 and ff % _CHUNK == 0
    assert sum(nr * nc for _, nr, _, nc in _W4_PIECES) == d * ff
    window = min(4096, max(256, sk // 4))
    dt = A_x.dtype

    wot, w4t = A_wo.T, B_w4.T
    hbm = pl.BlockSpec(memory_space=pltpu.HBM)
    return pl.pallas_call(
        _kernel,
        out_shape=jax.ShapeDtypeStruct(A_x.shape, dt),
        in_specs=[hbm] * 8,
        out_specs=pl.BlockSpec(memory_space=pltpu.VMEM),
        scratch_shapes=[
            pltpu.VMEM(A_x.shape, dt),
            pltpu.VMEM(gate_w.shape, dt),
            pltpu.VMEM((hkv, window, dh), dt),
            pltpu.VMEM((hkv, window, dh), dt),
            pltpu.VMEM(A_wq.shape, dt),
            pltpu.VMEM(wot.shape, dt),
            pltpu.VMEM(B_w3.shape, dt),
            pltpu.VMEM((_ROWS, hidden), jnp.float32),
            pltpu.VMEM((_ROWS, hidden), jnp.float32),
            pltpu.VMEM((_ROWS, ff), jnp.float32),
            pltpu.VMEM((_ROWS, d), jnp.float32),
            pltpu.SemaphoreType.DMA(()),
            *[pltpu.VMEM((nr, nc), dt) for _, nr, _, nc in _W4_PIECES],
        ],
        compiler_params=pltpu.CompilerParams(vmem_limit_bytes=64 * 2**20),
    )(A_x, gate_w, A_k_cache, A_v_cache, A_wq, wot, B_w3, w4t)
```

```python
import jax
import jax.numpy as jnp
from jax import lax
import jax.experimental.pallas as pl
import jax.experimental.pallas.tpu as pltpu

_ROWS = 8
_CHUNK = 512

_W4_PIECES = (
    (0, 576, 0, 2560),
    (0, 576, 2560, 1024),
    (256, 320, 3584, 1024),
    (128, 128, 3584, 1024),
    (0, 128, 3584, 512),
    (0, 128, 4096, 512),
)


def _dot(a, b):
    return jnp.dot(a, b, preferred_element_type=jnp.float32)


def _dot_nt(a, b):
    return lax.dot_general(
        a, b, (((1,), (1,)), ((), ())), preferred_element_type=jnp.float32
    )


def _kernel(
    x_hbm, gw_hbm, k_hbm, v_hbm, wq_hbm, wot_hbm, w3_hbm, w4t_hbm,
    out_ref,
    x_buf, gw_buf, k_buf, v_buf, wq_buf, wot_buf, w3_buf,
    q_buf, o_buf, h_buf, acc_buf, last_sem, *w4_bufs,
):
    f32, bf16 = jnp.float32, jnp.bfloat16
    hkv, window, dh = k_buf.shape
    d, ff = w3_buf.shape
    pair = 2 * dh

    def w4_copy(i, sem):
        r0, nr, c0, nc = _W4_PIECES[i]
        src = w4t_hbm.at[pl.ds(r0, nr), pl.ds(c0, nc)]
        return pltpu.make_async_copy(src, w4_bufs[i], sem)

    def mlp_down(i, copy):
        r0, nr, c0, nc = _W4_PIECES[i]
        hidden = h_buf[:, c0:c0 + nc].astype(bf16)
        partial = acc_buf[:, r0:r0 + nr]
        copy.wait()
        total = partial + _dot_nt(hidden, w4_bufs[i][...])
        if c0 + nc == ff:
            out_ref[0, :, r0:r0 + nr] = total[0:1].astype(out_ref.dtype)
        else:
            acc_buf[:, r0:r0 + nr] = total

    def chunk(i):
        return pl.ds(pl.multiple_of(i * _CHUNK, _CHUNK), _CHUNK)

    n_early = len(_W4_PIECES) - 1
    last_copy = w4_copy(n_early, last_sem)

    def all_but_last_piece(sems):
        def copy(src, dst, i):
            return pltpu.make_async_copy(src, dst, sems.at[i])

        recent = pl.ds(k_hbm.shape[2] - window, window)
        q_copies = (
            copy(wq_hbm, wq_buf, 0),
            copy(x_hbm, x_buf, 0),
            copy(gw_hbm, gw_buf, 0),
        )
        kv_copies = (
            copy(k_hbm.at[0, :, recent, :], k_buf, 1),
            copy(v_hbm.at[0, :, recent, :], v_buf, 1),
        )
        wo_copy = copy(wot_hbm, wot_buf, 2)
        w3_copy = copy(w3_hbm, w3_buf, 3)
        w4_copies = [w4_copy(i, sems.at[4 + i]) for i in range(n_early)]
        for c in (*q_copies, *kv_copies, wo_copy, w3_copy, *w4_copies, last_copy):
            c.start()

        for c in q_copies:
            c.wait()
        x = x_buf[0].astype(f32)
        gw = gw_buf[...].astype(f32).reshape(1, d)
        gate = jax.nn.sigmoid(jnp.sum(x * gw, axis=-1, keepdims=True))

        centered = x - jnp.mean(x, axis=-1, keepdims=True)
        var = jnp.mean(centered * centered, axis=-1, keepdims=True)
        normed = centered / jnp.sqrt(var + 1e-5)
        normed_rows = jnp.broadcast_to(normed, (_ROWS, d)).astype(bf16)
        x_rows = jnp.broadcast_to(x, (_ROWS, d)).astype(bf16)

        def q_step(i, carry):
            q_buf[:, chunk(i)] = _dot(x_rows, wq_buf[:, chunk(i)])
            return carry

        lax.fori_loop(0, hkv * pair // _CHUNK, q_step, None)

        for c in kv_copies:
            c.wait()
        row = lax.broadcasted_iota(jnp.int32, (_ROWS, dh), 0)

        def head_step(h, carry):
            even = pl.ds(pl.multiple_of(h * pair, pair), dh)
            odd = pl.ds(pl.multiple_of(h * pair + dh, dh), dh)
            q = jnp.where(row == 0, q_buf[:, even], q_buf[:, odd])
            s = _dot_nt(q.astype(bf16), k_buf[h]) * dh ** -0.5
            e = jnp.exp(s - jnp.max(s, axis=-1, keepdims=True))
            denom = jnp.sum(e, axis=-1, keepdims=True)
            o = _dot(e.astype(bf16), v_buf[h]) / denom
            o_buf[:, even] = jnp.where(row == 0, o, 0.0)
            o_buf[:, odd] = jnp.where(row == 1, o, 0.0)
            return carry

        lax.fori_loop(0, hkv, head_step, None)

        wo_copy.wait()

        def wo_step(i, acc):
            return acc + _dot_nt(o_buf[:, chunk(i)].astype(bf16), wot_buf[:, chunk(i)])

        attn = lax.fori_loop(
            0, hkv * pair // _CHUNK, wo_step, jnp.zeros((_ROWS, d), f32)
        )
        mixed = gate * (attn[0:1] + attn[1:2]) + (1.0 - gate) * x
        acc_buf[...] = jnp.broadcast_to(mixed, (_ROWS, d))

        w3_copy.wait()

        def up_step(i, carry):
            pre = _dot(normed_rows, w3_buf[:, chunk(i)])
            h_buf[:, chunk(i)] = (1.0 - gate) * jax.nn.gelu(pre, approximate=True)
            return carry

        lax.fori_loop(0, ff // _CHUNK, up_step, None)
        for i, c in enumerate(w4_copies):
            mlp_down(i, c)

    pl.run_scoped(all_but_last_piece, pltpu.SemaphoreType.DMA((4 + n_early,)))
    mlp_down(n_early, last_copy)


@jax.jit
def pallas_gated_mix__sliding_block_cached__mixer_s_mlp__decode_kernel(
    A_x: jax.Array,
    A_k_cache: jax.Array,
    A_v_cache: jax.Array,
    A_wq: jax.Array,
    A_wo: jax.Array,
    B_x: jax.Array,
    B_w1: jax.Array,
    B_w2: jax.Array,
    B_w3: jax.Array,
    B_w4: jax.Array,
    gate_w: jax.Array,
):
    del B_x, B_w1, B_w2
    b, sq, d = A_x.shape
    _, hkv, sk, dh = A_k_cache.shape
    ff = B_w3.shape[1]
    hidden = 2 * hkv * dh
    assert (b, sq) == (1, 1)
    assert A_wq.shape == (d, hidden) and hidden % _CHUNK == 0 and ff % _CHUNK == 0
    assert sum(nr * nc for _, nr, _, nc in _W4_PIECES) == d * ff
    window = min(4096, max(256, sk // 4))
    dt = A_x.dtype

    wot, w4t = A_wo.T, B_w4.T
    hbm = pl.BlockSpec(memory_space=pltpu.HBM)
    return pl.pallas_call(
        _kernel,
        out_shape=jax.ShapeDtypeStruct(A_x.shape, dt),
        in_specs=[hbm] * 8,
        out_specs=pl.BlockSpec(memory_space=pltpu.VMEM),
        scratch_shapes=[
            pltpu.VMEM(A_x.shape, dt),
            pltpu.VMEM(gate_w.shape, dt),
            pltpu.VMEM((hkv, window, dh), dt),
            pltpu.VMEM((hkv, window, dh), dt),
            pltpu.VMEM(A_wq.shape, dt),
            pltpu.VMEM(wot.shape, dt),
            pltpu.VMEM(B_w3.shape, dt),
            pltpu.VMEM((_ROWS, hidden), jnp.float32),
            pltpu.VMEM((_ROWS, hidden), jnp.float32),
            pltpu.VMEM((_ROWS, ff), jnp.float32),
            pltpu.VMEM((_ROWS, d), jnp.float32),
            pltpu.SemaphoreType.DMA(()),
            *[pltpu.VMEM((nr, nc), dt) for _, nr, _, nc in _W4_PIECES],
        ],
        compiler_params=pltpu.CompilerParams(vmem_limit_bytes=64 * 2**20),
    )(A_x, gate_w, A_k_cache, A_v_cache, A_wq, wot, B_w3, w4t)
```
